```python
import jax
import jax.numpy as jnp

def _softmax(x, axis=-1):
    return jax.nn.softmax(x, axis=axis)
def _gelu(x):
    return jax.nn.gelu(x, approximate=True)
def _silu(x):
    return jax.nn.silu(x)
def _sigmoid(x):
    return jax.nn.sigmoid(x)
def _layernorm(x, axis=-1, eps=1e-5):
    m = jnp.mean(x, axis=axis, keepdims=True)
    v = jnp.var(x, axis=axis, keepdims=True)
    return (x - m) / jnp.sqrt(v + eps)
def _scatter_add(tgt, idx, src, axis=0):
    return tgt.at[idx].add(src)
def _segment_sum(src, seg, n):
    return jax.ops.segment_sum(src, seg, n)
class _Rng:
    def __init__(self, key):
        self._k = key
    def _next(self):
        self._k, sub = jax.random.split(self._k)
        return sub
    def normal(self, shape):
        return jax.random.normal(self._next(), shape, dtype=jnp.bfloat16)
    def randint(self, lo, hi, shape):
        return jax.random.randint(self._next(), shape, lo, hi, dtype=jnp.int32)
    def uniform(self, shape, lo=0.0, hi=1.0):
        return jax.random.uniform(self._next(), shape, jnp.bfloat16, lo, hi)
    def permutation(self, n):
        return jax.random.permutation(self._next(), n)


kernel_name = 'standalone__structured_sparse_n_m__ragged'

def setup_inputs():
    _rng = _Rng(jax.random.key(int.from_bytes(__import__("os").urandom(4), "little")))
    _w = (lambda a: (lambda t: t.astype(jnp.bfloat16) if jnp.issubdtype(t.dtype, jnp.floating) else t)(jnp.asarray(a)))
    B, S, D = 16, 4096, 576
    assert D % 4 == 0, "d_model must be divisible by M=4 for 2:4 sparsity"
    return {
        "x": _w((lambda *s: _rng.normal(s) * 0.05)(B, S, D)),
        "w": _w((lambda *s: _rng.normal(s) * 0.05)(D, D)),
        "b": _w((lambda *s: _rng.normal(s) * 0.05)(D)),
    }

def reference(x, w, b):
    B, S, D = x.shape
    N, M = 2, 4
    G = D // M
    wg = w.reshape(G, M, D)
    mag = jnp.abs(wg)
    order = jnp.argsort(mag, 1)
    thr = jnp.take_along_axis(mag, order[:, M - N:M - N + 1, :], 1)
    mask = (lambda x, dt: x.astype(dt))(mag >= thr, w.dtype)
    wp = (wg * mask).reshape(D, D)
    return jnp.einsum("bsd,df->bsf", x, wp) + b
```

```python
import functools

import jax
import jax.numpy as jnp
import jax.experimental.pallas as pl
import jax.experimental.pallas.tpu as pltpu

_LANES = 128
_RAMP = (512, 1024, 2560)
_BODY = 6144
_OUT_CHUNKS = (2048, 2048, 1024, 512, 256, 128, 128)
_IN_CHUNKS = (2048, 2048, 2048)
_DOT = 512
_XPAD = _LANES


def _prune_2_of_4(wv):
    rows, cols = wv.shape
    words = pltpu.bitcast(wv, jnp.int32).reshape(rows // 16, 8, cols)
    a = pltpu.bitcast(jax.lax.shift_left(words, 16) & 0x7FFF0000, jnp.float32)
    c = pltpu.bitcast(words & 0x7FFF0000, jnp.float32)
    hi = jnp.maximum(a, c)
    lo = jnp.minimum(a, c)
    hi_n = pltpu.roll(hi, 7, 1)
    lo_n = pltpu.roll(lo, 7, 1)
    thr = jnp.maximum(jnp.minimum(hi, hi_n), jnp.maximum(lo, lo_n))
    even = (jax.lax.broadcasted_iota(jnp.int32, words.shape, 1) & 1) == 0
    thr = jnp.where(even, thr, pltpu.roll(thr, 1, 1))
    keep = jnp.where(a < thr, 0, 0xFFFF) | jnp.where(c < thr, 0, -0x10000)
    return pltpu.bitcast((words & keep).reshape(rows // 2, cols), jnp.bfloat16)


def _offsets(sizes):
    return [sum(sizes[:k]) for k in range(len(sizes))]


def _kernel(x_hbm, w_hbm, b_hbm, o_hbm,
            x_ramp, o_ramp, x_buf, o_buf, w_buf, b_buf, wt_ref,
            xr_sem, or_sem, x_sem, o_sem, wb_sem, order_sem):
    batch, d, seq = x_hbm.shape
    d_pad = wt_ref.shape[1]
    ramp_cols = sum(_RAMP)
    n_body = (batch * seq - ramp_cols) // _BODY
    ramp_off, out_off, in_off = _offsets(_RAMP), _offsets(_OUT_CHUNKS), _offsets(_IN_CHUNKS)
    copy = pltpu.make_async_copy

    def hbm_cols(ref, col, n):
        start = col % seq
        if not isinstance(start, int):
            start = pl.multiple_of(start, _LANES)
        return ref.at[col // seq, :, pl.ds(start, n)]

    def x_ramp_copy(k):
        return copy(hbm_cols(x_hbm, ramp_off[k], _RAMP[k]),
                    x_ramp.at[:, pl.ds(ramp_off[k], _RAMP[k])], xr_sem.at[k])

    def o_ramp_copy(k):
        return copy(o_ramp.at[:, pl.ds(ramp_off[k], _RAMP[k])],
                    hbm_cols(o_hbm, ramp_off[k], _RAMP[k]), or_sem.at[k])

    def x_copy(i, slot, j):
        return copy(hbm_cols(x_hbm, ramp_cols + i * _BODY + in_off[j], _IN_CHUNKS[j]),
                    x_buf.at[slot, :, pl.ds(in_off[j], _IN_CHUNKS[j])], x_sem.at[slot])

    def o_copy(i, slot, j):
        return copy(o_buf.at[slot, :, pl.ds(out_off[j], _OUT_CHUNKS[j])],
                    hbm_cols(o_hbm, ramp_cols + i * _BODY + out_off[j], _OUT_CHUNKS[j]),
                    o_sem.at[slot])

    def wait_slot(buf, sem, slot):
        view = buf.at[slot, :, pl.ds(0, _BODY)]
        copy(view, view, sem.at[slot]).wait()

    def start_in_order(copies):
        for n, cp in enumerate(copies):
            if n:
                pl.semaphore_signal(order_sem, 1)
                pl.semaphore_wait(order_sem, 1)
            cp.start()

    def linear(xv):
        row = jax.lax.broadcasted_iota(jnp.int32, (d_pad - d, xv.shape[1]), 0)
        ones = jnp.where(row == 0, 1.0, 0.0).astype(xv.dtype)
        acc = jnp.dot(wt_ref[...], jnp.concatenate([xv, ones], axis=0),
                      preferred_element_type=jnp.float32)
        return acc.astype(o_buf.dtype)

    b_copy = copy(b_hbm, b_buf, wb_sem.at[0])
    w_copy = copy(w_hbm, w_buf, wb_sem.at[1])
    start_in_order(
        [b_copy, w_copy]
        + [x_ramp_copy(k) for k in range(len(_RAMP))]
        + [x_copy(i, i, j) for i in range(2) for j in range(len(_IN_CHUNKS))])
    b_copy.wait()
    w_copy.wait()

    bias = b_buf[...].astype(jnp.float32).reshape(1, d)
    row = jax.lax.broadcasted_iota(jnp.int32, (d_pad - d, d), 0)
    bias_rows = jnp.where(row == 0, bias, 0.0).astype(w_buf.dtype)
    wt_ref[...] = jnp.concatenate([_prune_2_of_4(w_buf[...]), bias_rows], axis=0).T

    for k, n in enumerate(_RAMP):
        x_ramp_copy(k).wait()
        for c0 in range(ramp_off[k], ramp_off[k] + n, _DOT):
            o_ramp[:, pl.ds(c0, _DOT)] = linear(x_ramp[:, pl.ds(c0, _DOT)])
    start_in_order([o_ramp_copy(k) for k in range(len(_RAMP))])

    def body(i, carry):
        slot = i % 2
        wait_slot(x_buf, x_sem, slot)

        @pl.when(i >= 2)
        def _():
            wait_slot(o_buf, o_sem, slot)

        for j, n in enumerate(_OUT_CHUNKS):
            width = min(_DOT, n)
            for c0 in range(out_off[j], out_off[j] + n, width):
                o_buf[slot, :, pl.ds(c0, width)] = linear(x_buf[slot, :, pl.ds(c0, width)])
            o_copy(i, slot, j).start()
        for j in range(len(_IN_CHUNKS)):
            @pl.when(i + 2 < n_body)
            def _():
                x_copy(i + 2, slot, j).start()
        return carry

    jax.lax.fori_loop(0, n_body, body, 0)

    for k in range(len(_RAMP)):
        o_ramp_copy(k).wait()
    wait_slot(o_buf, o_sem, (n_body - 2) % 2)
    wait_slot(o_buf, o_sem, (n_body - 1) % 2)


@jax.jit
def pallas_standalone__structured_sparse_n_m__ragged_kernel(
    x: jax.Array,
    w: jax.Array,
    b: jax.Array,
):
    batch, seq, d = x.shape
    ramp_cols = sum(_RAMP)
    d_pad = pl.cdiv(d + 1, _LANES) * _LANES
    assert d % 16 == 0 and d % _LANES != 0
    assert seq == 4096 and (batch * seq - ramp_cols) % _BODY == 0
    dt = x.dtype

    out_t = pl.pallas_call(
        _kernel,
        in_specs=[pl.BlockSpec(memory_space=pl.ANY)] * 3,
        out_specs=pl.BlockSpec(memory_space=pl.ANY),
        out_shape=jax.ShapeDtypeStruct((batch, d, seq), dt),
        scratch_shapes=[
            pltpu.VMEM((d, ramp_cols + _XPAD), dt),
            pltpu.VMEM((d, ramp_cols), dt),
            pltpu.VMEM((2, d, _BODY + _XPAD), dt),
            pltpu.VMEM((2, d, _BODY), dt),
            pltpu.VMEM((d, d), w.dtype),
            pltpu.VMEM((d,), b.dtype),
            pltpu.VMEM((d, d_pad), w.dtype),
            pltpu.SemaphoreType.DMA((len(_RAMP),)),
            pltpu.SemaphoreType.DMA((len(_RAMP),)),
            pltpu.SemaphoreType.DMA((2,)),
            pltpu.SemaphoreType.DMA((2,)),
            pltpu.SemaphoreType.DMA((2,)),
            pltpu.SemaphoreType.REGULAR(()),
        ],
        compiler_params=pltpu.CompilerParams(vmem_limit_bytes=64 * 1024 * 1024),
    )(jnp.transpose(x, (0, 2, 1)), w, b)
    return jnp.transpose(out_t, (0, 2, 1))
```

```python
import functools

import jax
import jax.numpy as jnp
import jax.experimental.pallas as pl
import jax.experimental.pallas.tpu as pltpu

_LANES = 128
_RAMP = (512, 1024, 2560)
_BODY = 6144
_OUT_CHUNKS = (2048, 2048, 1024, 512, 256, 128, 128)
_IN_CHUNKS = (2048, 2048, 2048)
_DOT = 512
_XPAD = _LANES


def _prune_2_of_4(wv):
    rows, cols = wv.shape
    words = pltpu.bitcast(wv, jnp.int32).reshape(rows // 16, 8, cols)
    a = pltpu.bitcast(jax.lax.shift_left(words, 16) & 0x7FFF0000, jnp.float32)
    c = pltpu.bitcast(words & 0x7FFF0000, jnp.float32)
    hi = jnp.maximum(a, c)
    lo = jnp.minimum(a, c)
    hi_n = pltpu.roll(hi, 7, 1)
    lo_n = pltpu.roll(lo, 7, 1)
    thr = jnp.maximum(jnp.minimum(hi, hi_n), jnp.maximum(lo, lo_n))
    even = (jax.lax.broadcasted_iota(jnp.int32, words.shape, 1) & 1) == 0
    thr = jnp.where(even, thr, pltpu.roll(thr, 1, 1))
    keep = jnp.where(a < thr, 0, 0xFFFF) | jnp.where(c < thr, 0, -0x10000)
    return pltpu.bitcast((words & keep).reshape(rows // 2, cols), jnp.bfloat16)


def _offsets(sizes):
    return [sum(sizes[:k]) for k in range(len(sizes))]


def _kernel(x_hbm, w_hbm, b_hbm, o_hbm,
            x_ramp, o_ramp, x_buf, o_buf, w_buf, b_buf, wt_ref,
            xr_sem, or_sem, x_sem, o_sem, wb_sem, order_sem):
    batch, d, seq = x_hbm.shape
    d_pad = wt_ref.shape[1]
    ramp_cols = sum(_RAMP)
    n_body = (batch * seq - ramp_cols) // _BODY
    ramp_off, out_off, in_off = _offsets(_RAMP), _offsets(_OUT_CHUNKS), _offsets(_IN_CHUNKS)
    copy = pltpu.make_async_copy

    def hbm_cols(ref, col, n):
        start = col % seq
        if not isinstance(start, int):
            start = pl.multiple_of(start, _LANES)
        return ref.at[col // seq, :, pl.ds(start, n)]

    def x_ramp_copy(k):
        return copy(hbm_cols(x_hbm, ramp_off[k], _RAMP[k]),
                    x_ramp.at[:, pl.ds(ramp_off[k], _RAMP[k])], xr_sem.at[k])

    def o_ramp_copy(k):
        return copy(o_ramp.at[:, pl.ds(ramp_off[k], _RAMP[k])],
                    hbm_cols(o_hbm, ramp_off[k], _RAMP[k]), or_sem.at[k])

    def x_copy(i, slot, j):
        return copy(hbm_cols(x_hbm, ramp_cols + i * _BODY + in_off[j], _IN_CHUNKS[j]),
                    x_buf.at[slot, :, pl.ds(in_off[j], _IN_CHUNKS[j])], x_sem.at[slot])

    def o_copy(i, slot, j):
        return copy(o_buf.at[slot, :, pl.ds(out_off[j], _OUT_CHUNKS[j])],
                    hbm_cols(o_hbm, ramp_cols + i * _BODY + out_off[j], _OUT_CHUNKS[j]),
                    o_sem.at[slot])

    def wait_slot(buf, sem, slot):
        view = buf.at[slot, :, pl.ds(0, _BODY)]
        copy(view, view, sem.at[slot]).wait()

    def start_in_order(copies):
        for n, cp in enumerate(copies):
            if n:
                pl.semaphore_signal(order_sem, 1)
                pl.semaphore_wait(order_sem, 1)
            cp.start()

    def linear(xv):
        row = jax.lax.broadcasted_iota(jnp.int32, (d_pad - d, xv.shape[1]), 0)
        ones = jnp.where(row == 0, 1.0, 0.0).astype(xv.dtype)
        acc = jnp.dot(wt_ref[...], jnp.concatenate([xv, ones], axis=0),
                      preferred_element_type=jnp.float32)
        return acc.astype(o_buf.dtype)

    b_copy = copy(b_hbm, b_buf, wb_sem.at[0])
    w_copy = copy(w_hbm, w_buf, wb_sem.at[1])
    start_in_order(
        [b_copy, w_copy]
        + [x_ramp_copy(k) for k in range(len(_RAMP))]
        + [x_copy(i, i, j) for i in range(2) for j in range(len(_IN_CHUNKS))])
    b_copy.wait()
    w_copy.wait()

    bias = b_buf[...].astype(jnp.float32).reshape(1, d)
    row = jax.lax.broadcasted_iota(jnp.int32, (d_pad - d, d), 0)
    bias_rows = jnp.where(row == 0, bias, 0.0).astype(w_buf.dtype)
    wt_ref[...] = jnp.concatenate([_prune_2_of_4(w_buf[...]), bias_rows], axis=0).T

    for k, n in enumerate(_RAMP):
        x_ramp_copy(k).wait()
        for c0 in range(ramp_off[k], ramp_off[k] + n, _DOT):
            o_ramp[:, pl.ds(c0, _DOT)] = linear(x_ramp[:, pl.ds(c0, _DOT)])
    start_in_order([o_ramp_copy(k) for k in range(len(_RAMP))])

    def body(i, carry):
        slot = i % 2
        wait_slot(x_buf, x_sem, slot)

        @pl.when(i >= 2)
        def _():
            wait_slot(o_buf, o_sem, slot)

        for j, n in enumerate(_OUT_CHUNKS):
            width = min(_DOT, n)
            for c0 in range(out_off[j], out_off[j] + n, width):
                o_buf[slot, :, pl.ds(c0, width)] = linear(x_buf[slot, :, pl.ds(c0, width)])
            o_copy(i, slot, j).start()
        for j in range(len(_IN_CHUNKS)):
            @pl.when(i + 2 < n_body)
            def _():
                x_copy(i + 2, slot, j).start()
        return carry

    jax.lax.fori_loop(0, n_body, body, 0)

    for k in range(len(_RAMP)):
        o_ramp_copy(k).wait()
    wait_slot(o_buf, o_sem, (n_body - 2) % 2)
    wait_slot(o_buf, o_sem, (n_body - 1) % 2)


@jax.jit
def pallas_standalone__structured_sparse_n_m__ragged_kernel(
    x: jax.Array,
    w: jax.Array,
    b: jax.Array,
):
    batch, seq, d = x.shape
    ramp_cols = sum(_RAMP)
    d_pad = pl.cdiv(d + 1, _LANES) * _LANES
    assert d % 16 == 0 and d % _LANES != 0
    n_body, rem = divmod(batch * seq - ramp_cols, _BODY)
    assert rem == 0 and n_body >= 2 and ramp_cols <= seq
    assert sum(_IN_CHUNKS) == sum(_OUT_CHUNKS) == _BODY
    for chunks in (_IN_CHUNKS, _OUT_CHUNKS):
        for i in range(n_body):
            for off, n in zip(_offsets(chunks), chunks):
                assert (ramp_cols + i * _BODY + off) % seq + n <= seq
    dt = x.dtype

    out_t = pl.pallas_call(
        _kernel,
        in_specs=[pl.BlockSpec(memory_space=pl.ANY)] * 3,
        out_specs=pl.BlockSpec(memory_space=pl.ANY),
        out_shape=jax.ShapeDtypeStruct((batch, d, seq), dt),
        scratch_shapes=[
            pltpu.VMEM((d, ramp_cols + _XPAD), dt),
            pltpu.VMEM((d, ramp_cols), dt),
            pltpu.VMEM((2, d, _BODY + _XPAD), dt),
            pltpu.VMEM((2, d, _BODY), dt),
            pltpu.VMEM((d, d), w.dtype),
            pltpu.VMEM((d,), b.dtype),
            pltpu.VMEM((d, d_pad), w.dtype),
            pltpu.SemaphoreType.DMA((len(_RAMP),)),
            pltpu.SemaphoreType.DMA((len(_RAMP),)),
            pltpu.SemaphoreType.DMA((2,)),
            pltpu.SemaphoreType.DMA((2,)),
            pltpu.SemaphoreType.DMA((2,)),
            pltpu.SemaphoreType.REGULAR(()),
        ],
        compiler_params=pltpu.CompilerParams(vmem_limit_bytes=64 * 1024 * 1024),
    )(jnp.transpose(x, (0, 2, 1)), w, b)
    return jnp.transpose(out_t, (0, 2, 1))
```
